```python
import jax
import jax.numpy as jnp

def _softmax(x, axis=-1):
    return jax.nn.softmax(x, axis=axis)

def _gelu(x):
    return jax.nn.gelu(x, approximate=True)

def _silu(x):
    return jax.nn.silu(x)

def _sigmoid(x):
    return jax.nn.sigmoid(x)

def _layernorm(x, axis=-1, eps=1e-05):
    m = jnp.mean(x, axis=axis, keepdims=True)
    v = jnp.var(x, axis=axis, keepdims=True)
    return (x - m) / jnp.sqrt(v + eps)

def _scatter_add(tgt, idx, src, axis=0):
    return tgt.at[idx].add(src)

def _segment_sum(src, seg, n):
    return jax.ops.segment_sum(src, seg, n)

class _Rng:

    def __init__(self, key):
        self._k = key

    def _next(self):
        self._k, sub = jax.random.split(self._k)
        return sub

    def normal(self, shape):
        return jax.random.normal(self._next(), shape, dtype=jnp.bfloat16)

    def randint(self, lo, hi, shape):
        return jax.random.randint(self._next(), shape, lo, hi, dtype=jnp.int32)

    def uniform(self, shape, lo=0.0, hi=1.0):
        return jax.random.uniform(self._next(), shape, jnp.bfloat16, lo, hi)

    def permutation(self, n):
        return jax.random.permutation(self._next(), n)
kernel_name = 'adaLN_cond__sliding_block_cached__glu_gated_swiglu__decode'

def setup_inputs():
    _rng = _Rng(jax.random.key(int.from_bytes(__import__("os").urandom(4), "little")))
    _w = lambda a: (lambda t: t.astype(jnp.bfloat16) if jnp.issubdtype(t.dtype, jnp.floating) else t)(jnp.asarray(a))

    def _A_setup():
        B, Sq, D = (2, 1, 512)
        Hq, Hkv, Sk, Dh = (32, 32, 16384, 128)
        assert Hq % Hkv == 0, (Hq, Hkv)
        return {'x': _w((lambda *s: _rng.normal(s) * 0.05)(B, Sq, D)), 'k_cache': _w((lambda *s: _rng.normal(s) * 0.05)(B, Hkv, Sk, Dh)), 'v_cache': _w((lambda *s: _rng.normal(s) * 0.05)(B, Hkv, Sk, Dh)), 'wq': _w((lambda *s: _rng.normal(s) * 0.05)(D, Hq * Dh) * D ** (-0.5)), 'wo': _w((lambda *s: _rng.normal(s) * 0.05)(Hq * Dh, D) * (Hq * Dh) ** (-0.5))}
    _A_in = _A_setup()

    def _B_setup():
        B, S, D, F = (2, 1, 512, 1376)
        return {'x': _w((lambda *s: _rng.normal(s) * 0.05)(B, S, D)), 'w1': _w((lambda *s: _rng.normal(s) * 0.05)(D, F) * (2.0 / D) ** 0.5), 'w3': _w((lambda *s: _rng.normal(s) * 0.05)(D, F) * (2.0 / D) ** 0.5), 'w2': _w((lambda *s: _rng.normal(s) * 0.05)(F, D) * (2.0 / F) ** 0.5)}
    _B_in = _B_setup()
    return {'A_x': _A_in['x'], 'A_k_cache': _A_in['k_cache'], 'A_v_cache': _A_in['v_cache'], 'A_wq': _A_in['wq'], 'A_wo': _A_in['wo'], 'B_x': _B_in['x'], 'B_w1': _B_in['w1'], 'B_w3': _B_in['w3'], 'B_w2': _B_in['w2'], 'c': _w((lambda *s: _rng.normal(s) * 0.05)(2, 512)), 'w_mod': _w((lambda *s: _rng.normal(s) * 0.05)(512, 6 * 512) * 512 ** (-0.5))}

def reference(A_x, A_k_cache, A_v_cache, A_wq, A_wo, B_x, B_w1, B_w3, B_w2, c, w_mod):

    def _A_ref(x, k_cache, v_cache, wq, wo):
        B, Sq, D = x.shape
        Hq, Dh = (32, 128)
        Hkv, Sk = (k_cache.shape[1], k_cache.shape[2])
        W = min(4096, max(256, Sk // 4))
        rep = Hq // Hkv
        q = (lambda x, *d: x.transpose(*d))((x @ wq).reshape(B, Sq, Hq, Dh), 0, 2, 1, 3)
        k = jnp.repeat(k_cache[:, :, Sk - W:, :], rep, axis=1)
        v = jnp.repeat(v_cache[:, :, Sk - W:, :], rep, axis=1)
        scores = jnp.einsum('bhqd,bhkd->bhqk', q, k) * Dh ** (-0.5)
        p = _softmax(scores, axis=-1)
        o = jnp.einsum('bhqk,bhkd->bhqd', p, v)
        return (lambda x, *d: x.transpose(*d))(o, 0, 2, 1, 3).reshape(B, Sq, Hq * Dh) @ wo

    def _B_ref(x, w1, w3, w2):
        gate = jnp.einsum('bsd,df->bsf', x, w1)
        up = jnp.einsum('bsd,df->bsf', x, w3)
        h = _silu(gate) * up
        out = jnp.einsum('bsf,fd->bsd', h, w2)
        return out
    x = A_x
    mod = (_silu(c) @ w_mod).reshape(c.shape[0], 6, 1, -1)
    sa, ca, ga, sb, cb, gb = (mod[:, 0].copy(), mod[:, 1].copy(), mod[:, 2].copy(), mod[:, 3].copy(), mod[:, 4].copy(), mod[:, 5].copy())
    h = _layernorm(x, axis=-1) * (1 + ca) + sa
    x = x + ga * _A_ref(h, A_k_cache, A_v_cache, A_wq, A_wo)
    h = _layernorm(x, axis=-1) * (1 + cb) + sb
    x = x + gb * _B_ref(h, B_w1, B_w3, B_w2)
    return x
```

```python
import jax
import jax.numpy as jnp
from jax import lax
from jax.experimental import pallas as pl
from jax.experimental.pallas import tpu as pltpu

BF = jnp.bfloat16
F32 = jnp.float32

D = 512
DH = 128
NH = 32
NBH = 64
SK = 16384
W = 4096
FF = 1376
G = 8
NG = NBH // G
RB = 128
NR = W // RB
NU = NG * NR
PR = 16
NS = RB // PR
T_WM, T_WQ, T_WO = 12, 28, 44
NT = NU - T_WO
T_V = NU + T_WO // 2
FD = FF // 32

_NT = (((1,), (1,)), ((), ()))


def _ln(x):
    m = jnp.mean(x, axis=-1, keepdims=True)
    d = x - m
    v = jnp.mean(d * d, axis=-1, keepdims=True)
    return d * lax.rsqrt(v + 1e-5)


def _silu(x):
    return x * (1.0 / (1.0 + jnp.exp(-x)))


def _rep(x2):
    n = x2.shape[1]
    return jnp.concatenate([jnp.broadcast_to(x2[0:1], (G, n)), jnp.broadcast_to(x2[1:2], (G, n))], axis=0)


def _shr(x, n):
    return lax.shift_right_logical(x, jnp.int32(n))


def make(NSEM=6, NKB=64, NVB=16, name="fused", w2cuts=(8, 24, 36, 40, 43), VCAP=4):
    T0 = T_WQ + NSEM - 1
    TEND = T_V + NSEM
    assert NSEM == 6

    def kern(x_hbm, c_hbm, wm_hbm, wq_hbm, k_hbm, v_hbm, wo_hbm, w1_hbm, w3_hbm, w2_hbm, o_ref,
             xb, cb, wm, wq, wo, w1, w3, w2, kbuf, vbuf, mod, o16, qs, sbuf, pbuf, linv, acc, att, sems):
        row8 = lax.broadcasted_iota(jnp.int32, (G, DH), 0)
        row16 = lax.broadcasted_iota(jnp.int32, (2 * G, DH), 0) & (G - 1)

        def wait_on(dst, sem):
            pltpu.make_async_copy(dst, dst, sem).wait()

        def unit_desc(src, buf, u, slot, sem, prio):
            g = _shr(u, 5)
            r = u & (NR - 1)
            h0 = (g & 1) * NH + _shr(g, 1) * G

            def go(s):
                pltpu.make_async_copy(
                    src.at[pl.ds(h0, G), pl.ds(pl.multiple_of(SK - W + r * RB + s * PR, PR), PR), :],
                    buf.at[slot, s], sem).start(priority=prio)
            return go

        def box_desc(src, dst, sem, at):
            def go(s):
                r0, c0 = at(s)
                r0, c0 = pl.multiple_of(r0, 8), pl.multiple_of(c0, D)
                pltpu.make_async_copy(src.at[:, pl.ds(r0, 8), pl.ds(c0, D)],
                                      dst.at[:, pl.ds(r0, 8), pl.ds(c0, D)], sem).start(priority=1)
            return go

        def start_f(src, dst, d, sem, prio):
            pltpu.make_async_copy(src.at[:, pl.ds(pl.multiple_of(d * 16, 16), 16), :],
                                  dst.at[pl.ds(2 * d, 2)], sem).start(priority=prio)

        def interleave(a, b, unroll):
            if unroll:
                for s in range(NS):
                    a(s)
                    b(s)
            else:
                def one(s, _):
                    a(s)
                    b(s)
                    return 0
                lax.fori_loop(0, NS, one, 0)

        def v_unit(n):
            m = n - NT
            return jnp.where(m < 0, n, NT + _shr(m, 1) + (m & 1) * (T_WO // 2))

        def qk(u, _):
            slot = u & (NKB - 1)
            g = _shr(u, 5)
            r = u & (NR - 1)
            b = g & 1
            q = qs[_shr(g, 1), pl.ds(pl.multiple_of(b * G, G), G), :].astype(BF)
            s = None
            for j in range(G):
                kj = kbuf[slot, :, j].reshape(RB, DH)
                res = lax.dot_general(q, kj, _NT, preferred_element_type=F32)
                s = res if s is None else jnp.where(row8 == j, res, s)
            sbuf[r] = s

            @pl.when(r == NR - 1)
            def _():
                sc = sbuf[...] * (DH ** -0.5)
                m = jnp.max(jnp.max(sc, axis=0), axis=-1, keepdims=True)
                e = jnp.exp(sc - m[None])
                l = jnp.sum(jnp.sum(e, axis=0), axis=-1, keepdims=True)
                pbuf[b] = e.astype(BF)
                linv[b] = jnp.broadcast_to(1.0 / l, (G, DH))
                acc[b] = jnp.zeros((G, DH), F32)
            return 0

        def pv(n, _):
            slot = n & (NVB - 1)
            u = v_unit(n)
            g = _shr(u, 5)
            r = u & (NR - 1)
            b = g & 1
            p = pbuf[b, r]
            s = None
            for j in range(G):
                vj = vbuf[slot, :, j].reshape(RB, DH)
                res = jnp.dot(p, vj, preferred_element_type=F32)
                s = res if s is None else jnp.where(row8 == j, res, s)
            acc[b] += s

            @pl.when(r == NR - 1)
            def _():
                o16[pl.ds(pl.multiple_of(b * G, G), G), :] = acc[b] * linv[b]

                @pl.when(b == 1)
                def _():
                    o = o16[...]
                    lhs = jnp.concatenate(
                        [jnp.where(row16 == j, o, 0.0).astype(BF) for j in range(G)], axis=1)
                    att[...] += jnp.dot(lhs, wo[_shr(g, 1)], preferred_element_type=F32)
            return 0

        def step(t, carry):
            kdone, vdone, si = carry
            sem = sems.at[si]
            ta = t - NSEM

            @pl.when(ta == 0)
            def _():
                wait_on(xb, sem)
                wait_on(cb, sem)

            @pl.when((ta >= 0) & (ta < NU))
            def _():
                wait_on(kbuf.at[ta & (NKB - 1)], sem)

            @pl.when((ta >= 0) & (ta < T_WM))
            def _():
                wait_on(wm.at[:, pl.ds(pl.multiple_of((ta & 1) * 64, 64), 64),
                              pl.ds(pl.multiple_of(_shr(ta, 1) * D, D), D)], sem)

            @pl.when((ta >= T_WM) & (ta < T_WQ))
            def _():
                wait_on(wq.at[:, pl.ds(pl.multiple_of((ta - T_WM) * 8, 8), 8), :], sem)

            @pl.when((ta >= T_WQ) & (ta < T_WO))
            def _():
                wait_on(wo.at[:, pl.ds(pl.multiple_of((ta - T_WQ) * 64, 64), 64), :], sem)

            @pl.when((ta >= T_WO) & (ta < NU))
            def _():
                wait_on(vbuf.at[(ta - T_WO) & (NVB - 1)], sem)

            @pl.when(ta >= NU)
            def _():
                wait_on(vbuf.at[pl.ds((NT + 2 * (ta - NU)) & (NVB - 1), 2)], sem)

            @pl.when(t == 0)
            def _():
                pltpu.make_async_copy(x_hbm, xb, sem).start()
                pltpu.make_async_copy(c_hbm, cb, sem).start()

            kd = unit_desc(k_hbm, kbuf, t, t & (NKB - 1), sem, 0)

            @pl.when((t >= T_WO) & (t < NU))
            def _():
                n = t - T_WO
                interleave(kd, unit_desc(v_hbm, vbuf, n, n & (NVB - 1), sem, 1), True)

            @pl.when(t < T_WM)
            def _():
                interleave(kd, box_desc(wm_hbm, wm, sem, lambda s: ((t & 1) * 64 + s * 8, _shr(t, 1) * D)), False)

            @pl.when((t >= T_WM) & (t < T_WQ))
            def _():
                interleave(kd, box_desc(wq_hbm, wq, sem, lambda s: ((t - T_WM) * 8, s * D)), False)

            @pl.when((t >= T_WQ) & (t < T_WO))
            def _():
                interleave(kd, box_desc(wo_hbm, wo, sem, lambda s: ((t - T_WQ) * 64 + s * 8, 0)), False)

            @pl.when((t >= NU) & (t < T_V))
            def _():
                n = NT + 2 * (t - NU)
                interleave(unit_desc(v_hbm, vbuf, v_unit(n), n & (NVB - 1), sem, 0),
                           unit_desc(v_hbm, vbuf, v_unit(n + 1), (n + 1) & (NVB - 1), sem, 1), False)

            @pl.when((t >= T_V) & (t < TEND - 1))
            def _():
                interleave(lambda s: start_f(w1_hbm, w1, (t - T_V) * NS + s, sem, 0),
                           lambda s: start_f(w3_hbm, w3, (t - T_V) * NS + s, sem, 1), False)

            @pl.when(t == TEND - 1)
            def _():
                for d in range((NSEM - 1) * NS, FD):
                    start_f(w1_hbm, w1, d, sem, 0)
                    start_f(w3_hbm, w3, d, sem, 1)
                for d in range(w2cuts[0]):
                    start_f(w2_hbm, w2, d, sem, d % 2)

            @pl.when(ta == T_WM - 1)
            def _():
                sc = _silu(_rep(cb[...].astype(F32))).astype(BF)

                def one(i, _):
                    c0 = pl.multiple_of(i * D, D)
                    y = None
                    for kb in range(4):
                        z = jnp.dot(sc[:, kb * DH:(kb + 1) * DH], wm[kb, :, pl.ds(c0, D)],
                                    preferred_element_type=F32)
                        y = z if y is None else y + z
                    mod[i] = y
                    return 0
                lax.fori_loop(0, 6, one, 0)
                att[...] = jnp.zeros(att.shape, F32)

            @pl.when(t == T0)
            def _():
                h = (_ln(_rep(xb[...].astype(F32))) * (1.0 + mod[1]) + mod[0]).astype(BF)

                def one(i, _):
                    q = None
                    for j in range(0, G, 4):
                        c0 = pl.multiple_of((i * G + j) * DH, 4 * DH)
                        y = None
                        for kb in range(4):
                            z = jnp.dot(h[:, kb * DH:(kb + 1) * DH], wq[kb, :, pl.ds(c0, 4 * DH)],
                                        preferred_element_type=F32)
                            y = z if y is None else y + z
                        for jj in range(4):
                            yj = y[:, jj * DH:(jj + 1) * DH]
                            q = yj if q is None else jnp.where(row16 == j + jj, yj, q)
                    qs[i] = q
                    return 0
                lax.fori_loop(0, NH // G, one, 0)

            ktgt = jnp.minimum(jnp.minimum(ta + 1, 2 * (t - T0 + 1)), NU)
            ktgt = jnp.maximum(ktgt, kdone)
            lax.fori_loop(kdone, ktgt, qk, 0)
            varr = jnp.where(ta < NU, ta - T_WO + 1, NT + 2 * (ta - NU + 1))
            vtgt = jnp.minimum(jnp.minimum(varr, ktgt & ~(NR - 1)), vdone + VCAP)
            vtgt = jnp.maximum(vtgt, vdone)
            vtgt = jnp.where(t == TEND - 1, NU, vtgt)
            lax.fori_loop(vdone, vtgt, pv, 0)
            return ktgt, vtgt, jnp.where(si == NSEM - 1, 0, si + 1)

        lax.fori_loop(0, TEND, step, (0, 0, 0))

        a = att[...]
        a16 = jnp.concatenate(
            [jnp.broadcast_to(jnp.sum(a[b * G:(b + 1) * G], axis=0, keepdims=True), (G, D)) for b in range(2)],
            axis=0)
        x1 = _rep(xb[...].astype(F32)) + mod[2] * a16
        h2 = (_ln(x1) * (1.0 + mod[4]) + mod[3]).astype(BF)

        def gate_up(d0, d1):
            n = (d1 - d0) * 32
            gt = lax.dot_general(h2, w1[2 * d0:2 * d1].reshape(n, D), _NT, preferred_element_type=F32)
            up = lax.dot_general(h2, w3[2 * d0:2 * d1].reshape(n, D), _NT, preferred_element_type=F32)
            return (_silu(gt) * up).astype(BF)

        acts = []
        for i in range(NSEM - 1):
            sem = sems.at[(TEND + i) % NSEM]
            wait_on(w1.at[pl.ds(2 * NS * i, 2 * NS)], sem)
            wait_on(w3.at[pl.ds(2 * NS * i, 2 * NS)], sem)
            if i + 1 < len(w2cuts):
                for d in range(w2cuts[i], w2cuts[i + 1]):
                    start_f(w2_hbm, w2, d, sem, d % 2)
            acts.append(gate_up(NS * i, NS * (i + 1)))
        sem = sems.at[(TEND - 1) % NSEM]
        d0 = (NSEM - 1) * NS
        wait_on(w1.at[pl.ds(2 * d0, 2 * (FD - d0))], sem)
        wait_on(w3.at[pl.ds(2 * d0, 2 * (FD - d0))], sem)
        wait_on(w2.at[pl.ds(0, 2 * w2cuts[0])], sem)
        acts.append(gate_up(d0, FD))
        act = jnp.concatenate(acts, axis=1)

        y = None
        for i, d1 in enumerate(w2cuts):
            d0 = w2cuts[i - 1] if i else 0
            if i:
                wait_on(w2.at[pl.ds(2 * d0, 2 * (d1 - d0))], sems.at[(TEND + i - 1) % NSEM])
            z = jnp.dot(act[:, 32 * d0:32 * d1], w2[2 * d0:2 * d1].reshape(32 * (d1 - d0), D),
                        preferred_element_type=F32)
            y = z if y is None else y + z
        out = x1 + mod[5] * y
        o_ref[...] = jnp.concatenate([out[0:1], out[G:G + 1]], axis=0).astype(o_ref.dtype)

    def f(A_x, A_k_cache, A_v_cache, A_wq, A_wo, B_x, B_w1, B_w3, B_w2, c, w_mod):
        hbm = pl.BlockSpec(memory_space=pltpu.HBM)
        sp = lambda w, s: w.reshape(s, w.shape[0] // s, w.shape[1])
        out = pl.pallas_call(
            kern,
            in_specs=[hbm] * 10,
            out_specs=pl.BlockSpec(memory_space=pltpu.VMEM),
            out_shape=jax.ShapeDtypeStruct((2, D), A_x.dtype),
            scratch_shapes=[
                pltpu.VMEM((2, D), BF), pltpu.VMEM((2, D), BF),
                pltpu.VMEM((4, DH, 6 * D), BF), pltpu.VMEM((4, DH, NH * DH), BF), pltpu.VMEM((4, G * DH, D), BF),
                pltpu.VMEM((2 * FD, 16, D), BF), pltpu.VMEM((2 * FD, 16, D), BF), pltpu.VMEM((2 * FD, 16, D), BF),
                pltpu.VMEM((NKB, NS, G, PR, DH), BF), pltpu.VMEM((NVB, NS, G, PR, DH), BF),
                pltpu.VMEM((6, 2 * G, D), F32), pltpu.VMEM((2 * G, DH), F32), pltpu.VMEM((NH // G, 2 * G, DH), F32),
                pltpu.VMEM((NR, G, DH), F32), pltpu.VMEM((2, NR, G, DH), BF), pltpu.VMEM((2, G, DH), F32),
                pltpu.VMEM((2, G, DH), F32), pltpu.VMEM((2 * G, D), F32),
                pltpu.SemaphoreType.DMA((NSEM,)),
            ],
            compiler_params=pltpu.CompilerParams(vmem_limit_bytes=64 * 1024 * 1024, disable_bounds_checks=True),
            name=name,
        )(A_x.reshape(2, D), c, sp(w_mod, 4), sp(A_wq, 4),
          A_k_cache.reshape(NBH, SK, DH), A_v_cache.reshape(NBH, SK, DH),
          sp(A_wo, 4), sp(B_w1.T, 2), sp(B_w3.T, 2), sp(B_w2, 2))
        return out.reshape(2, 1, D)
    return f


_impl = make()


@jax.jit
def pallas_adaLN_cond__sliding_block_cached__glu_gated_swiglu__decode_kernel(
    A_x: jax.Array,
    A_k_cache: jax.Array,
    A_v_cache: jax.Array,
    A_wq: jax.Array,
    A_wo: jax.Array,
    B_x: jax.Array,
    B_w1: jax.Array,
    B_w3: jax.Array,
    B_w2: jax.Array,
    c: jax.Array,
    w_mod: jax.Array,
):
    return _impl(A_x, A_k_cache, A_v_cache, A_wq, A_wo, B_x, B_w1, B_w3, B_w2, c, w_mod)
```

```python
import jax
import jax.numpy as jnp
from jax import lax
import jax.experimental.pallas as pl
import jax.experimental.pallas.tpu as pltpu

BF = jnp.bfloat16
F32 = jnp.float32

B = 2
D = 512
DH = 128
NH = 32
SK = 16384
W = min(4096, max(256, SK // 4))
FF = 1376
G = 8
RB = 128
NR = W // RB
NU = (B * NH // G) * NR
PR = 16
NS = RB // PR
FD = FF // 32

NSEM = 6
NKB = 64
NVB = 32
VCAP = 4

T_WM, T_WQ, T_WO = 12, 28, 44
T_Q = T_WQ + NSEM - 1
NT = NU - T_WO
C1 = T_WO // 2
E7 = NR - C1
T_F = NU + C1
T_END = T_F + NSEM
FM = (NSEM - 1) * NS
W2_SPLIT = 20
W2_CUT = 32
W2_ORDER = sorted([((i + 1) / W2_SPLIT, 0, i) for i in range(W2_SPLIT)]
                  + [((i + 1) / (FD - W2_SPLIT), 1, W2_SPLIT + i) for i in range(FD - W2_SPLIT)])

_NT_DIMS = (((1,), (1,)), ((), ()))


def _layernorm(x):
    m = jnp.mean(x, axis=-1, keepdims=True)
    d = x - m
    v = jnp.mean(d * d, axis=-1, keepdims=True)
    return d * lax.rsqrt(v + 1e-5)


def _silu(x):
    return x * (1.0 / (1.0 + jnp.exp(-x)))


def _rep(x2):
    n = x2.shape[1]
    return jnp.concatenate([jnp.broadcast_to(x2[0:1], (G, n)), jnp.broadcast_to(x2[1:2], (G, n))], axis=0)


def _shr(x, n):
    return lax.shift_right_logical(x, jnp.int32(n))


def _loop(n, fn):
    def body(i, carry):
        fn(i)
        return carry
    lax.fori_loop(0, n, body, 0)


def _v_unit(n):
    m = jnp.maximum(n - NT, 0)
    two = jnp.where((m & 1) == 0, NU - NR - C1, NU - NR + E7) + _shr(m, 1)
    return jnp.where(n < NT - E7, n, jnp.where(n < NT, n + C1, two))


def _kernel(x_hbm, c_hbm, wm_hbm, wq_hbm, k_hbm, v_hbm, wo_hbm, w1_hbm, w3_hbm, w2_hbm, o_ref,
            xb, cb, wm, wq, wo, w1, w3, w2, kbuf, vbuf,
            mod, o16, qs, sbuf, pbuf, linv, acc, att, sems, w2sems):
    row8 = lax.broadcasted_iota(jnp.int32, (G, DH), 0)
    row16 = lax.broadcasted_iota(jnp.int32, (2 * G, DH), 0) & (G - 1)
    first_row = lax.broadcasted_iota(jnp.int32, (G, D), 0) == 0

    def wait_on(dst, sem):
        pltpu.make_async_copy(dst, dst, sem).wait()

    def unit_copy(src, buf, u, slot, sem):
        g = _shr(u, 5)
        r = u & (NR - 1)
        h0 = (g & 1) * NH + _shr(g, 1) * G

        def desc(s):
            r0 = pl.multiple_of(SK - W + r * RB + s * PR, PR)
            return pltpu.make_async_copy(src.at[pl.ds(h0, G), pl.ds(r0, PR), :], buf.at[slot, s], sem)
        return desc

    def box_copy(src, dst, sem, at):
        def desc(s):
            r0, c0 = at(s)
            r0, c0 = pl.multiple_of(r0, 8), pl.multiple_of(c0, D)
            return pltpu.make_async_copy(src.at[:, pl.ds(r0, 8), pl.ds(c0, D)],
                                         dst.at[:, pl.ds(r0, 8), pl.ds(c0, D)], sem)
        return desc

    def wm_copy(i, sem):
        def at(s):
            d = i * NS + s
            rb = _shr(d * 43, 8)
            return rb * 8, (d - 6 * rb) * D
        return box_copy(wm_hbm, wm, sem, at)

    def f_copy(src, dst, d, sem):
        return pltpu.make_async_copy(src.at[:, pl.ds(pl.multiple_of(d * 16, 16), 16), :],
                                     dst.at[pl.ds(2 * d, 2)], sem)

    def start_pairs(a, b):
        for s in range(NS):
            a(s).start(priority=0)
            b(s).start(priority=1)

    def start_w2(lo, hi):
        for _, queue, d in W2_ORDER[lo:hi]:
            f_copy(w2_hbm, w2, d, w2sems.at[int(d >= W2_CUT)]).start(priority=queue)

    def qk(u, carry):
        slot = u & (NKB - 1)
        g = _shr(u, 5)
        r = u & (NR - 1)
        b = g & 1
        q = qs[_shr(g, 1), pl.ds(pl.multiple_of(b * G, G), G), :].astype(BF)
        s = None
        for j in range(G):
            kj = kbuf[slot, :, j].reshape(RB, DH)
            res = lax.dot_general(q, kj, _NT_DIMS, preferred_element_type=F32)
            s = res if s is None else jnp.where(row8 == j, res, s)
        sbuf[r] = s

        @pl.when(r == NR - 1)
        def _():
            sc = sbuf[...] * (DH ** -0.5)
            m = jnp.max(jnp.max(sc, axis=0), axis=-1, keepdims=True)
            e = jnp.exp(sc - m[None])
            l = jnp.sum(jnp.sum(e, axis=0), axis=-1, keepdims=True)
            pbuf[b] = e.astype(BF)
            linv[b] = jnp.broadcast_to(1.0 / l, (G, DH))
            acc[b] = jnp.zeros((G, DH), F32)
        return carry

    def pv(n, carry):
        slot = n & (NVB - 1)
        u = _v_unit(n)
        g = _shr(u, 5)
        r = u & (NR - 1)
        b = g & 1
        p = pbuf[b, r]
        s = None
        for j in range(G):
            vj = vbuf[slot, :, j].reshape(RB, DH)
            res = jnp.dot(p, vj, preferred_element_type=F32)
            s = res if s is None else jnp.where(row8 == j, res, s)
        acc[b] += s

        @pl.when(r == NR - 1)
        def _():
            o16[pl.ds(pl.multiple_of(b * G, G), G), :] = acc[b] * linv[b]

            @pl.when(b == 1)
            def _():
                o = o16[...]
                lhs = jnp.concatenate(
                    [jnp.where(row16 == j, o, 0.0).astype(BF) for j in range(G)], axis=1)
                att[...] += jnp.dot(lhs, wo[_shr(g, 1)], preferred_element_type=F32)
        return carry

    def project(lhs, w, c0):
        y = None
        for kb in range(4):
            z = jnp.dot(lhs[:, kb * DH:(kb + 1) * DH], w[kb, :, pl.ds(c0, D)], preferred_element_type=F32)
            y = z if y is None else y + z
        return y

    def modulation():
        sc = _silu(_rep(cb[...].astype(F32))).astype(BF)

        def one(i):
            mod[i] = project(sc, wm, pl.multiple_of(i * D, D))
        _loop(6, one)
        att[...] = jnp.zeros(att.shape, F32)

    def queries():
        h = (_layernorm(_rep(xb[...].astype(F32))) * (1.0 + mod[1]) + mod[0]).astype(BF)

        def one(i):
            q = None
            for j0 in range(0, G, 4):
                y = project(h, wq, pl.multiple_of((i * G + j0) * DH, D))
                for j in range(4):
                    yj = y[:, j * DH:(j + 1) * DH]
                    q = yj if q is None else jnp.where(row16 == j0 + j, yj, q)
            qs[i] = q
        _loop(NH // G, one)

    def step(t, carry):
        kdone, vdone, si = carry
        sem = sems.at[si]
        ta = t - NSEM

        @pl.when((ta >= 0) & (ta < NU))
        def _():
            wait_on(kbuf.at[ta & (NKB - 1)], sem)

        @pl.when((ta >= T_WO) & (ta < NU))
        def _():
            wait_on(vbuf.at[(ta - T_WO) & (NVB - 1)], sem)

        @pl.when((ta >= 0) & (ta < T_WO))
        def _():
            @pl.when(ta == 0)
            def _():
                wait_on(xb, sem)
                wait_on(cb, sem)

            @pl.when(ta < T_WM)
            def _():
                desc = wm_copy(ta, sem)
                _loop(NS, lambda s: desc(s).wait())

            @pl.when((ta >= T_WM) & (ta < T_WQ))
            def _():
                wait_on(wq.at[:, pl.ds(pl.multiple_of((ta - T_WM) * 8, 8), 8), :], sem)

            @pl.when(ta >= T_WQ)
            def _():
                wait_on(wo.at[:, pl.ds(pl.multiple_of((ta - T_WQ) * 64, 64), 64), :], sem)

        @pl.when(ta >= NU)
        def _():
            wait_on(vbuf.at[pl.ds((NT + 2 * (ta - NU)) & (NVB - 1), 2)], sem)

        k_desc = unit_copy(k_hbm, kbuf, t, t & (NKB - 1), sem)

        @pl.when((t >= T_WO) & (t < NU))
        def _():
            n = t - T_WO
            start_pairs(k_desc, unit_copy(v_hbm, vbuf, _v_unit(n), n & (NVB - 1), sem))

        @pl.when(t < T_WO)
        def _():
            @pl.when(t < T_WM)
            def _():
                start_pairs(k_desc, wm_copy(t, sem))

            @pl.when(t == 0)
            def _():
                pltpu.make_async_copy(x_hbm, xb, sem).start()
                pltpu.make_async_copy(c_hbm, cb, sem).start()

            @pl.when((t >= T_WM) & (t < T_WQ))
            def _():
                start_pairs(k_desc, box_copy(wq_hbm, wq, sem, lambda s: ((t - T_WM) * 8, s * D)))

            @pl.when(t >= T_WQ)
            def _():
                start_pairs(k_desc, box_copy(wo_hbm, wo, sem, lambda s: ((t - T_WQ) * 64 + s * 8, 0)))

            pl.when(ta == T_WM - 1)(modulation)
            pl.when(t == T_Q)(queries)

        @pl.when(t >= NU)
        def _():
            @pl.when(t < T_F)
            def _():
                n = NT + 2 * (t - NU)
                start_pairs(unit_copy(v_hbm, vbuf, _v_unit(n), n & (NVB - 1), sem),
                            unit_copy(v_hbm, vbuf, _v_unit(n + 1), (n + 1) & (NVB - 1), sem))

            @pl.when((t >= T_F) & (t < T_END - 1))
            def _():
                start_pairs(lambda s: f_copy(w1_hbm, w1, (t - T_F) * NS + s, sem),
                            lambda s: f_copy(w3_hbm, w3, (t - T_F) * NS + s, sem))

            @pl.when(t == T_END - 1)
            def _():
                for d in range(FM, FD):
                    f_copy(w1_hbm, w1, d, sem).start(priority=0)
                    f_copy(w3_hbm, w3, d, sem).start(priority=1)
                start_w2(0, 16)

        ktgt = jnp.minimum(jnp.minimum(ta + 1, (3 * (t - T_Q + 1)) >> 1), NU)
        ktgt = jnp.maximum(ktgt, kdone)
        lax.fori_loop(kdone, ktgt, qk, 0)
        arrived = jnp.where(ta < NU, ta - T_WO + 1, NT + 2 * (ta - NU + 1))
        ready = ktgt & ~(NR - 1)
        ready = jnp.where(ready == NU - NR, NT - E7, ready)
        vtgt = jnp.minimum(jnp.minimum(arrived, ready), vdone + VCAP)
        vtgt = jnp.maximum(vtgt, vdone)
        lax.fori_loop(vdone, vtgt, pv, 0)
        return ktgt, vtgt, jnp.where(si == NSEM - 1, 0, si + 1)

    lax.fori_loop(0, T_END, step, (0, 0, 0))

    def fold(a):
        return jnp.where(first_row, a[0:G], a[G:2 * G])

    a = att[...]
    attn = jnp.where(first_row, jnp.sum(a[0:G], axis=0, keepdims=True),
                     jnp.sum(a[G:2 * G], axis=0, keepdims=True))
    out = fold(_rep(xb[...].astype(F32))) + fold(mod[2]) * attn
    h2 = (_layernorm(out) * (1.0 + fold(mod[4])) + fold(mod[3])).astype(BF)

    acts = []
    for i in range(NSEM):
        d0, d1 = NS * i, (NS * (i + 1) if i < NSEM - 1 else FD)
        sem = sems.at[(T_F + i) % NSEM]
        wait_on(w1.at[pl.ds(2 * d0, 2 * (d1 - d0))], sem)
        wait_on(w3.at[pl.ds(2 * d0, 2 * (d1 - d0))], sem)
        start_w2(16 * (i + 1), 16 * (i + 2))
        n = 32 * (d1 - d0)
        gate = lax.dot_general(h2, w1[2 * d0:2 * d1].reshape(n, D), _NT_DIMS, preferred_element_type=F32)
        up = lax.dot_general(h2, w3[2 * d0:2 * d1].reshape(n, D), _NT_DIMS, preferred_element_type=F32)
        acts.append((_silu(gate) * up).astype(BF))
    act = jnp.concatenate(acts, axis=1)

    gb = fold(mod[5])
    for i, (d0, d1) in enumerate(((0, W2_CUT), (W2_CUT, FD))):
        wait_on(w2.at[pl.ds(2 * d0, 2 * (d1 - d0))], w2sems.at[i])
        out = out + gb * jnp.dot(act[:, 32 * d0:32 * d1], w2[2 * d0:2 * d1].reshape(32 * (d1 - d0), D),
                                 preferred_element_type=F32)
    o_ref[...] = out[0:B].astype(o_ref.dtype)


def _split_rows(w, parts):
    return w.reshape(parts, w.shape[0] // parts, w.shape[1])


@jax.jit
def pallas_adaLN_cond__sliding_block_cached__glu_gated_swiglu__decode_kernel(
    A_x: jax.Array,
    A_k_cache: jax.Array,
    A_v_cache: jax.Array,
    A_wq: jax.Array,
    A_wo: jax.Array,
    B_x: jax.Array,
    B_w1: jax.Array,
    B_w3: jax.Array,
    B_w2: jax.Array,
    c: jax.Array,
    w_mod: jax.Array,
):
    del B_x
    assert A_k_cache.shape == (B, NH, SK, DH) and B_w1.shape == (D, FF)
    out = pl.pallas_call(
        _kernel,
        in_specs=[pl.BlockSpec(memory_space=pltpu.HBM)] * 10,
        out_specs=pl.BlockSpec(memory_space=pltpu.VMEM),
        out_shape=jax.ShapeDtypeStruct((B, D), A_x.dtype),
        scratch_shapes=[
            pltpu.VMEM((B, D), BF),
            pltpu.VMEM((B, D), BF),
            pltpu.VMEM((4, D // 4, 6 * D), BF),
            pltpu.VMEM((4, D // 4, NH * DH), BF),
            pltpu.VMEM((4, G * DH, D), BF),
            pltpu.VMEM((2 * FD, 16, D), BF),
            pltpu.VMEM((2 * FD, 16, D), BF),
            pltpu.VMEM((2 * FD, 16, D), BF),
            pltpu.VMEM((NKB, NS, G, PR, DH), BF),
            pltpu.VMEM((NVB, NS, G, PR, DH), BF),
            pltpu.VMEM((6, 2 * G, D), F32),
            pltpu.VMEM((2 * G, DH), F32),
            pltpu.VMEM((NH // G, 2 * G, DH), F32),
            pltpu.VMEM((NR, G, DH), F32),
            pltpu.VMEM((B, NR, G, DH), BF),
            pltpu.VMEM((B, G, DH), F32),
            pltpu.VMEM((B, G, DH), F32),
            pltpu.VMEM((2 * G, D), F32),
            pltpu.SemaphoreType.DMA((NSEM,)),
            pltpu.SemaphoreType.DMA((2,)),
        ],
        compiler_params=pltpu.CompilerParams(vmem_limit_bytes=64 * 1024 * 1024),
        name="adaln_window_attn_swiglu_decode",
    )(A_x.reshape(B, D), c, _split_rows(w_mod, 4), _split_rows(A_wq, 4),
      A_k_cache.reshape(B * NH, SK, DH), A_v_cache.reshape(B * NH, SK, DH),
      _split_rows(A_wo, 4), _split_rows(B_w1.T, 2), _split_rows(B_w3.T, 2), _split_rows(B_w2, 2))
    return out.reshape(B, 1, D)
```
